```python
import os as _os
_os.environ.setdefault("JAX_PLATFORMS", "cpu")
import jax
import jax.numpy as jnp

def _softmax(x, axis=-1):
    return jax.nn.softmax(x, axis=axis)
def _gelu(x):
    return jax.nn.gelu(x, approximate=True)
def _silu(x):
    return jax.nn.silu(x)
def _sigmoid(x):
    return jax.nn.sigmoid(x)
def _layernorm(x, axis=-1, eps=1e-5):
    m = jnp.mean(x, axis=axis, keepdims=True)
    v = jnp.var(x, axis=axis, keepdims=True)
    return (x - m) / jnp.sqrt(v + eps)
def _scatter_add(tgt, idx, src, axis=0):
    return tgt.at[idx].add(src)
def _segment_sum(src, seg, n):
    return jax.ops.segment_sum(src, seg, n)
class _Rng:
    def __init__(self, key):
        self._k = key
    def _next(self):
        self._k, sub = jax.random.split(self._k)
        return sub
    def normal(self, shape):
        return jax.random.normal(self._next(), shape, dtype=jnp.bfloat16)
    def randint(self, lo, hi, shape):
        return jax.random.randint(self._next(), shape, lo, hi, dtype=jnp.int32)
    def uniform(self, shape, lo=0.0, hi=1.0):
        return jax.random.uniform(self._next(), shape, jnp.bfloat16, lo, hi)
    def permutation(self, n):
        return jax.random.permutation(self._next(), n)


kernel_name = 'interleave_layers__mha_block__dense_activation_mish__prompt'

def setup_inputs():
    _rng = _Rng(jax.random.key(int.from_bytes(__import__("os").urandom(4), "little")))
    _w = (lambda a: (lambda t: t.astype(jnp.bfloat16) if jnp.issubdtype(t.dtype, jnp.floating) else t)(jnp.asarray(a)))
    def _A_setup():
        B, S, D, H = 1, 2048, 512, 32
        return {
            "x": _w((lambda *s: _rng.normal(s) * 0.05)(B, S, D)),
            "wqkv": _w((lambda *s: _rng.normal(s) * 0.05)(D, 3 * D)),
            "wo": _w((lambda *s: _rng.normal(s) * 0.05)(D, D)),
        }
    _A_in = _A_setup()

    def _B_setup():
        B, S, D, F = 1, 2048, 512, 1792
        return {
            "x": _w((lambda *s: _rng.normal(s) * 0.05)(B, S, D)),
            "w1": _w((lambda *s: _rng.normal(s) * 0.4)(D, F) * (D ** -0.5)),
            "b1": _w((lambda *s: _rng.normal(s) * 0.4)(F)),
            "w2": _w((lambda *s: _rng.normal(s) * 0.4)(F, D) * (F ** -0.5)),
        }
    _B_in = _B_setup()

    return {
        "A_x": _A_in["x"],
        "A_wqkv": _A_in["wqkv"],
        "A_wo": _A_in["wo"],
        "B_x": _B_in["x"],
        "B_w1": _B_in["w1"],
        "B_b1": _B_in["b1"],
        "B_w2": _B_in["w2"],
    }

def reference(A_x, A_wqkv, A_wo, B_x, B_w1, B_b1, B_w2):
    def _A_ref(x, wqkv, wo):
        B, S, D = x.shape
        H = 32
        Dh = D // H
        qkv = (lambda x, *d: x.transpose(*d))((x @ wqkv).reshape(B, S, 3, H, Dh), 2, 0, 3, 1, 4)
        q, k, v = qkv[0], qkv[1], qkv[2]
        scores = jnp.einsum("bhqd,bhkd->bhqk", q, k) * (Dh ** -0.5)
        p = _softmax(scores, axis=-1)
        o = jnp.einsum("bhqk,bhkd->bhqd", p, v)
        return (lambda x, *d: x.transpose(*d))(o, 0, 2, 1, 3).reshape(B, S, D) @ wo

    def _B_ref(x, w1, b1, w2):
        h = jnp.einsum("bsd,df->bsf", x, w1) + b1
        sp = jnp.log1p(jnp.exp(-jnp.abs(h))) + jnp.where(h > 0, h, jnp.zeros_like(h))
        act = h * jnp.tanh(sp)
        return jnp.einsum("bsf,fd->bsd", act, w2)

    x = A_x
    x = x + _A_ref(_layernorm(x, axis=-1), A_wqkv, A_wo)
    x = x + _B_ref(_layernorm(x, axis=-1), B_w1, B_b1, B_w2)
    x = x + _A_ref(_layernorm(x, axis=-1), A_wqkv, A_wo)
    x = x + _B_ref(_layernorm(x, axis=-1), B_w1, B_b1, B_w2)
    return x
```

```python
import jax
import jax.numpy as jnp
from jax import lax
import jax.experimental.pallas as pl
import jax.experimental.pallas.tpu as pltpu

S, D, H, DH, F = 2048, 512, 32, 16, 1792
NQ = 512
NB = S // NQ
KC = 128
NC = S // KC
NP = 4
MP = NQ // NP
LAG = 2
DEFER = 8
NSLOT = 8
LOG2E = 1.4426950408889634
QSCALE = (DH ** -0.5) * LOG2E
L_LO = 2.0 ** -60
L_HI = 2.0 ** 60
EPS = 1e-5

F32 = jnp.float32
BF16 = jnp.bfloat16
U32 = jnp.uint32


def _ln(x):
    m = jnp.mean(x, axis=-1, keepdims=True)
    xc = x - m
    v = jnp.mean(xc * xc, axis=-1, keepdims=True)
    return (xc * lax.rsqrt(v + EPS)).astype(BF16)


def _rcp(d):
    r = pltpu.reciprocal(d, approx=True)
    return r * (2.0 - d * r)


def _mish(h):
    e = jnp.exp2(jnp.minimum(h, 20.0) * LOG2E)
    n = e * (e + 2.0)
    return h * n * _rcp(n + 2.0)


def _pack(x):
    return pltpu.bitcast(x, U32)


def _unpack(x):
    return pltpu.bitcast(x, BF16)


def _half(i, m):
    return i // 2 if isinstance(i, int) else pl.multiple_of(i // 2, m // 2)


def _transposed(w):
    return w.astype(F32).T.astype(BF16)


def _dot(a, b):
    return jnp.dot(a, b, preferred_element_type=F32)


def _kernel(x_hbm, wqkv_hbm, wo_hbm, w1_hbm, b1_hbm, w2_hbm, out_hbm,
            xin_ref, wqkv_ref, wo_ref, w1_ref, b1_ref, w2_ref, outs_ref,
            x_ref, wqvT_ref, woT_ref, qT_ref, k_ref, vT_ref, oT_ref, p_ref, xn0_ref,
            sem_in, sem_out):
    def copy(src, dst, sem):
        return pltpu.make_async_copy(src, dst, sem)

    def cp_rows(r0, n, i):
        return copy(x_hbm.at[pl.ds(r0, n), :], xin_ref.at[pl.ds(r0, n), :], sem_in.at[i])

    def cp_wqkv(i):
        return copy(wqkv_hbm.at[:, pl.ds(i * D, D)], wqkv_ref.at[:, pl.ds(i * D, D)], sem_in.at[3 + i])

    cp_xa, cp_xb, cp_xc = cp_rows(0, MP, 0), cp_rows(MP, NQ - MP, 1), cp_rows(NQ, S - NQ, 2)
    cp_wq, cp_wk, cp_wv = cp_wqkv(0), cp_wqkv(1), cp_wqkv(2)
    cp_wo = copy(wo_hbm, wo_ref, sem_in.at[6])
    cp_w1 = copy(w1_hbm, w1_ref, sem_in.at[7])
    cp_b1 = copy(b1_hbm, b1_ref, sem_in.at[8])
    cp_w2 = copy(w2_hbm, w2_ref, sem_in.at[9])

    def cp_out(t):
        rows = pl.ds(t * NQ, NQ)
        return copy(outs_ref.at[rows, :], out_hbm.at[rows, :], sem_out.at[t])

    def kproj(xn, t0, buf):
        kk = _dot(xn, wqkv_ref[:, D:2 * D])
        k_ref[buf, pl.ds(_half(t0, MP), MP // 2), :] = _pack(kk.astype(BF16))

    def qvproj(xn, t0, buf):
        qv = lax.dot_general(wqvT_ref[...], xn, (((1,), (1,)), ((), ())), preferred_element_type=F32)
        qT_ref[buf, :, pl.ds(t0, MP)] = _pack((qv[0:D] * QSCALE).astype(BF16))
        vT_ref[buf, :, pl.ds(t0, MP)] = _pack(qv[D:2 * D].astype(BF16))

    def load_piece(p):
        if p == 0:
            cp_xa.wait()
            cp_xb.start()
        elif p == 1:
            cp_xb.wait()
        elif p == NP:
            cp_xc.wait()
            cp_wo.start()
            cp_w1.start()
            cp_b1.start()
            cp_w2.start()
        elif p == 2 * NP:
            cp_wo.wait()
            woT_ref[...] = _transposed(wo_ref[...])
        x = xin_ref[p * MP:(p + 1) * MP, :].astype(F32)
        x_ref[p * MP:(p + 1) * MP, :] = x
        return _ln(x)

    cp_xa.start()
    cp_wk.start()
    xn = load_piece(0)
    cp_wk.wait()
    cp_wq.start()
    cp_wv.start()
    pending = []
    for p in range(S // MP):
        kproj(xn, p * MP, 0)
        if p == 2:
            cp_wq.wait()
            cp_wv.wait()
            cp_xc.start()
            wqvT_ref[0:D, :] = _transposed(wqkv_ref[:, 0:D])
            wqvT_ref[D:2 * D, :] = _transposed(wqkv_ref[:, 2 * D:3 * D])
        xn_next = load_piece(p + 1) if p + 1 < S // MP else None
        pending.append(xn)
        if p >= 2:
            for i, xp in enumerate(pending):
                qvproj(xp, (p + 1 - len(pending) + i) * MP, 0)
            pending = []
        xn = xn_next
    cp_w1.wait()
    cp_b1.wait()
    cp_w2.wait()

    def attn_fast(buf, q0):
        def group(g, bad):
            l0 = pl.multiple_of(g * 128, 128)

            def head_rows(j, packed):
                if packed:
                    return pl.ds(pl.multiple_of(g * 64 + j * (DH // 2), DH // 2), DH // 2)
                return pl.ds(pl.multiple_of(g * 128 + j * DH, DH), DH)

            def q_weights(j):
                qh = _unpack(qT_ref[buf, head_rows(j, True), pl.ds(q0, NQ)])
                parts = [jnp.zeros((DH * j, NQ), BF16)] if j > 0 else []
                parts.append(qh)
                if j < 7:
                    parts.append(jnp.zeros((DH * (7 - j), NQ), BF16))
                return jnp.concatenate(parts, axis=0)

            seq = [(j, c) for j in range(8) for c in range(NC)]
            n = len(seq)
            events = []
            for i in range(n):
                events.append((True, i))
                if 0 <= i - LAG < n - DEFER:
                    events.append((False, i - LAG))
            events += [(False, i) for i in range(n - DEFER, n)]

            unsafe = jnp.zeros((1, NQ), F32)
            row_sums = {}
            for is_qk, i in events:
                j, c = seq[i]
                if is_qk:
                    if c == 0:
                        w = q_weights(j)
                        l = jnp.zeros((8, NQ), F32)
                    kk = _unpack(k_ref[buf, pl.ds(c * KC // 2, KC // 2), pl.ds(l0, 128)])
                    p = jnp.exp2(_dot(kk, w))
                    l = l + jnp.sum(p.reshape(KC // 8, 8, NQ), axis=0)
                    p_ref[i % NSLOT] = _pack(p.astype(BF16))
                    if c == NC - 1:
                        row_sums[j] = l
                else:
                    if c == 0:
                        o = jnp.zeros((DH, NQ), F32)
                    vv = _unpack(vT_ref[buf, head_rows(j, True), pl.ds(c * KC, KC)])
                    o = o + _dot(vv, _unpack(p_ref[i % NSLOT]))
                    if c == NC - 1:
                        lsum = jnp.sum(row_sums.pop(j), axis=0, keepdims=True)
                        ok = (lsum >= L_LO) & (lsum <= L_HI)
                        unsafe = jnp.maximum(unsafe, jnp.where(ok, 0.0, 1.0))
                        oT_ref[head_rows(j, False), :] = (o * _rcp(lsum)).astype(BF16)
            return jnp.maximum(bad, jnp.max(unsafe))
        return lax.fori_loop(0, D // 128, group, jnp.float32(0.0))

    def attn_safe(buf, q0):
        ck = 512

        def head(h, carry):
            l0 = pl.multiple_of((h // 8) * 128, 128)
            r0 = pl.multiple_of(h * DH, DH)
            qg = _unpack(qT_ref[buf, pl.ds(_half(l0, 128), 64), pl.ds(q0, NQ)])
            in_head = lax.broadcasted_iota(jnp.int32, (128, NQ), 0) // DH == h % 8
            w = jnp.where(in_head, qg, jnp.zeros_like(qg))

            def scores(i):
                k0 = pl.multiple_of(i * ck, ck)
                return _dot(_unpack(k_ref[buf, pl.ds(_half(k0, ck), ck // 2), pl.ds(l0, 128)]), w)

            m = lax.fori_loop(
                0, S // ck, lambda i, m: jnp.maximum(m, jnp.max(scores(i), axis=0, keepdims=True)),
                jnp.full((1, NQ), -jnp.inf, F32))

            def accumulate(i, ol):
                p = jnp.exp2(scores(i) - m)
                vv = _unpack(vT_ref[buf, pl.ds(_half(r0, DH), DH // 2), pl.ds(pl.multiple_of(i * ck, ck), ck)])
                return ol[0] + _dot(vv, p.astype(BF16)), ol[1] + jnp.sum(p, axis=0, keepdims=True)
            o, l = lax.fori_loop(0, S // ck, accumulate,
                                 (jnp.zeros((DH, NQ), F32), jnp.zeros((1, NQ), F32)))
            oT_ref[pl.ds(r0, DH), :] = (o / l).astype(BF16)
            return carry
        lax.fori_loop(0, H, head, 0)

    def layer_block(layer, t):
        t0 = pl.multiple_of(t * NQ, NQ)
        bad = attn_fast(layer, t0)

        @pl.when(bad > 0.0)
        def _():
            attn_safe(layer, t0)

        def rows(i):
            return pl.ds(pl.multiple_of(t0 + i * MP, MP), MP)

        ys = [_dot(woT_ref[...], oT_ref[:, i * MP:(i + 1) * MP]).T for i in range(NP)]
        hs = []
        for i in range(NP):
            x = x_ref[rows(i), :] + ys[i]
            x_ref[rows(i), :] = x
            hs.append(_dot(_ln(x), w1_ref[...]))
        b1 = b1_ref[...].astype(F32).reshape(1, F)
        act = jnp.concatenate([_mish(h + b1).astype(BF16) for h in hs], axis=0)
        x = x_ref[pl.ds(t0, NQ), :] + _dot(act, w2_ref[...])
        outs_ref[pl.ds(t0, NQ), :] = x.astype(outs_ref.dtype)
        x_ref[pl.ds(t0, NQ), :] = x
        xn0_ref[...] = _ln(x[0:MP])

        @pl.when(layer == 0)
        def _():
            for i in range(NP):
                xn = xn0_ref[...] if i == 0 else _ln(x_ref[rows(i), :])
                ti = pl.multiple_of(t0 + i * MP, MP)
                kproj(xn, ti, 1)
                qvproj(xn, ti, 1)

        @pl.when(layer == 1)
        def _():
            cp_out(t).start()

    def step(i, carry):
        layer_block(i // NB, i % NB)
        return carry
    lax.fori_loop(0, 2 * NB, step, 0)
    for t in range(NB):
        cp_out(t).wait()


@jax.jit
def pallas_interleave_layers__mha_block__dense_activation_mish__prompt_kernel(
    A_x, A_wqkv, A_wo, B_x, B_w1, B_b1, B_w2,
):
    del B_x
    hbm = pl.BlockSpec(memory_space=pl.ANY)
    out = pl.pallas_call(
        _kernel,
        out_shape=jax.ShapeDtypeStruct((S, D), BF16),
        in_specs=[hbm] * 6,
        out_specs=hbm,
        scratch_shapes=[
            pltpu.VMEM((S, D), BF16),
            pltpu.VMEM((D, 3 * D), BF16),
            pltpu.VMEM((D, D), BF16),
            pltpu.VMEM((D, F), BF16),
            pltpu.VMEM((F,), BF16),
            pltpu.VMEM((F, D), BF16),
            pltpu.VMEM((S, D), BF16),
            pltpu.VMEM((S, D), F32),
            pltpu.VMEM((2 * D, D), BF16),
            pltpu.VMEM((D, D), BF16),
            pltpu.VMEM((2, D // 2, S), U32),
            pltpu.VMEM((2, S // 2, D), U32),
            pltpu.VMEM((2, D // 2, S), U32),
            pltpu.VMEM((D, NQ), BF16),
            pltpu.VMEM((NSLOT, KC // 2, NQ), U32),
            pltpu.VMEM((MP, D), BF16),
            pltpu.SemaphoreType.DMA((10,)),
            pltpu.SemaphoreType.DMA((NB,)),
        ],
        compiler_params=pltpu.CompilerParams(vmem_limit_bytes=100 * 1024 * 1024),
    )(A_x.reshape(S, D), A_wqkv, A_wo, B_w1, B_b1, B_w2)
    return out.reshape(1, S, D)
```
